```python
import jax
import jax.numpy as jnp

def _softmax(x, axis=-1):
    return jax.nn.softmax(x, axis=axis)

def _gelu(x):
    return jax.nn.gelu(x, approximate=True)

def _silu(x):
    return jax.nn.silu(x)

def _sigmoid(x):
    return jax.nn.sigmoid(x)

def _layernorm(x, axis=-1, eps=1e-05):
    m = jnp.mean(x, axis=axis, keepdims=True)
    v = jnp.var(x, axis=axis, keepdims=True)
    return (x - m) / jnp.sqrt(v + eps)

def _scatter_add(tgt, idx, src, axis=0):
    return tgt.at[idx].add(src)

def _segment_sum(src, seg, n):
    return jax.ops.segment_sum(src, seg, n)

class _Rng:

    def __init__(self, key):
        self._k = key

    def _next(self):
        self._k, sub = jax.random.split(self._k)
        return sub

    def normal(self, shape):
        return jax.random.normal(self._next(), shape, dtype=jnp.bfloat16)

    def randint(self, lo, hi, shape):
        return jax.random.randint(self._next(), shape, lo, hi, dtype=jnp.int32)

    def uniform(self, shape, lo=0.0, hi=1.0):
        return jax.random.uniform(self._next(), shape, jnp.bfloat16, lo, hi)

    def permutation(self, n):
        return jax.random.permutation(self._next(), n)
kernel_name = 'sequential_preLN__memory_aug_recurrent_mem_tr__moe_arch_mod__prompt'

def setup_inputs():
    _rng = _Rng(jax.random.key(int.from_bytes(__import__("os").urandom(4), "little")))
    _w = lambda a: (lambda t: t.astype(jnp.bfloat16) if jnp.issubdtype(t.dtype, jnp.floating) else t)(jnp.asarray(a))

    def _A_setup():
        B, S, Dm = (1, 2048, 512)
        H, Dh = (32, 128)
        M, seg = (8, 32)
        seg = min(seg, S)
        S = S // seg * seg
        return {'x': _w((lambda *s: _rng.normal(s) * 0.05)(B, S, Dm)), 'mem0': _w((lambda *s: _rng.normal(s) * 0.05)(B, M, Dm)), 'Wq': _w((lambda *s: _rng.normal(s) * 0.05)(Dm, H, Dh) * Dm ** (-0.5)), 'Wk': _w((lambda *s: _rng.normal(s) * 0.05)(Dm, H, Dh) * Dm ** (-0.5)), 'Wv': _w((lambda *s: _rng.normal(s) * 0.05)(Dm, H, Dh) * Dm ** (-0.5)), 'Wo': _w((lambda *s: _rng.normal(s) * 0.05)(H, Dh, Dm) * (H * Dh) ** (-0.5)), 'seg_len': seg}
    _A_in = _A_setup()

    def _B_setup():
        B, S, D, F, C = (1, 2048, 512, 1792, 2)
        return {'x': _w((lambda *s: _rng.normal(s) * 0.05)(B, S, D)), 'w_r': _w((lambda *s: _rng.normal(s) * 0.05)(D)), 'w_gate': _w((lambda *s: _rng.normal(s) * 0.05)(D, F)), 'w_up': _w((lambda *s: _rng.normal(s) * 0.05)(D, F)), 'w_down': _w((lambda *s: _rng.normal(s) * 0.05)(F, D))}
    _B_in = _B_setup()
    return {'A_x': _A_in['x'], 'A_mem0': _A_in['mem0'], 'A_Wq': _A_in['Wq'], 'A_Wk': _A_in['Wk'], 'A_Wv': _A_in['Wv'], 'A_Wo': _A_in['Wo'], 'A_seg_len': _A_in['seg_len'], 'B_x': _B_in['x'], 'B_w_r': _B_in['w_r'], 'B_w_gate': _B_in['w_gate'], 'B_w_up': _B_in['w_up'], 'B_w_down': _B_in['w_down']}

def reference(A_x, A_mem0, A_Wq, A_Wk, A_Wv, A_Wo, A_seg_len, B_x, B_w_r, B_w_gate, B_w_up, B_w_down):

    def _A_ref(x, mem0, Wq, Wk, Wv, Wo, seg_len):
        B, S, Dm = x.shape
        H, Dh = (Wq.shape[1], Wq.shape[2])
        M = mem0.shape[1]
        scale = Dh ** (-0.5)
        n_seg = S // seg_len
        L = M + seg_len
        idx = jnp.arange(L)
        mask = (idx[:, None] < M) | (idx[:, None] >= idx[None, :])
        mem = mem0
        outs = []
        for s in range(n_seg):
            xs = x[:, s * seg_len:(s + 1) * seg_len, :].copy()
            h = jnp.concatenate([mem, xs], axis=1)
            q = jnp.einsum('btd,dhe->bhte', h, Wq)
            k = jnp.einsum('btd,dhe->bhte', h, Wk)
            v = jnp.einsum('btd,dhe->bhte', h, Wv)
            scores = jnp.einsum('bhqe,bhke->bhqk', q, k) * scale
            scores = jnp.where(mask[None, None], scores, -1000000000.0)
            p = _softmax(scores, axis=-1)
            o = jnp.einsum('bhqk,bhke->bhqe', p, v)
            o = jnp.einsum('bhte,hed->btd', o, Wo)
            mem = o[:, :M, :].copy()
            outs.append(o[:, M:, :])
        return jnp.concatenate(outs, axis=1)

    def _B_ref(x, w_r, w_gate, w_up, w_down):
        B, S, D = x.shape
        C = 2
        r = x @ w_r
        idx = jnp.argsort(-r, axis=-1)[:, :C]
        idx_e = jnp.repeat(idx.reshape(B, C, 1), D, axis=2)
        x_sel = jnp.take_along_axis(x, idx_e, axis=1)
        g = _silu(x_sel @ w_gate)
        u = x_sel @ w_up
        y = g * u @ w_down
        r_sel = _sigmoid(jnp.take_along_axis(r, idx, axis=1))
        y = y * r_sel.reshape(B, C, 1)
        b_off = (jnp.arange(B) * S).reshape(B, 1)
        flat_idx = (idx + b_off).reshape(B * C)
        zero = (x * 0.0).reshape(B * S, D)
        upd = _scatter_add(zero, flat_idx, y.reshape(B * C, D), axis=0)
        return x + upd.reshape(B, S, D)
    x = A_x
    h = x + _A_ref(_layernorm(x, axis=-1), A_mem0, A_Wq, A_Wk, A_Wv, A_Wo, A_seg_len)
    h2 = h + _B_ref(_layernorm(h, axis=-1), B_w_r, B_w_gate, B_w_up, B_w_down)
    return h2
```

```python
import functools
import math

import numpy as np
import jax
import jax.numpy as jnp
from jax import lax
import jax.experimental.pallas as pl
import jax.experimental.pallas.tpu as pltpu

BF = jnp.bfloat16
F32 = jnp.float32
U32 = jnp.uint32
NN = (((1,), (0,)), ((), ()))
NT = (((1,), (1,)), ((), ()))


def _rb(v):
    return v.astype(BF).astype(F32)


def _layernorm(x):
    n = x.shape[-1]
    mean = jnp.sum(x, axis=-1, keepdims=True) * (1.0 / n)
    c = x - mean
    var = jnp.sum(c * c, axis=-1, keepdims=True) * (1.0 / n)
    eps = float(np.float32(1e-5).astype(BF))
    den = _rb(jnp.sqrt(_rb(_rb(var) + eps)))
    return _rb(_rb(x - _rb(mean)) * (1.0 / den))


def _dot(a, b, dn=NN):
    return lax.dot_general(a, b, dn, preferred_element_type=F32)


def _make_kernel(S, D, H, E, M, T, F, cfg):
    G = H // 2
    L = M + T
    NSEG = S // T
    scale = float(E) ** -0.5
    fill_masked = float(np.float32(-1e9).astype(BF)) / scale
    c_exp = scale * math.log2(math.e)

    def kernel(x_hbm, mem_hbm, wq_hbm, wk_hbm, wv_hbm, wo_hbm, wr_hbm, wg_hbm, wu_hbm, wd_hbm,
               out_hbm,
               x_v, mem_v, wr_v, stg, wqkv, wo_v, wg_v, wu_v, wd_v,
               lhs_s, o_s, ao_s, h_s, out_v, r_s, fill_s, wrb_s,
               sem_w, sem_m):
        cx = pltpu.make_async_copy(x_hbm, x_v, sem_m.at[0])
        cm = pltpu.make_async_copy(mem_hbm, mem_v, sem_m.at[1])
        cr = pltpu.make_async_copy(wr_hbm, wr_v, sem_m.at[2])
        cx.start(); cm.start(); cr.start()

        def wcopy(g, m):
            w = (wq_hbm, wk_hbm, wv_hbm)[m]
            return pltpu.make_async_copy(w.bitcast(U32).at[:, g, :], stg.at[3 * g + m], sem_w.at[3 * g + m])

        for g in range(G):
            for m in range(3):
                wcopy(g, m).start()
        cwo = [pltpu.make_async_copy(wo_hbm.bitcast(U32).at[:, pl.ds(128 * i, 128)], wo_v.at[i], sem_m.at[3 + i])
               for i in range(D // 128)]
        for c in cwo:
            c.start()
        cg = pltpu.make_async_copy(wg_hbm, wg_v, sem_m.at[8])
        cu = pltpu.make_async_copy(wu_hbm, wu_v, sem_m.at[9])
        cd = pltpu.make_async_copy(wd_hbm, wd_v, sem_m.at[10])
        cg.start(); cu.start(); cd.start()

        ri = lax.broadcasted_iota(jnp.int32, (2 * L, 2 * L), 0)
        ci = lax.broadcasted_iota(jnp.int32, (2 * L, 2 * L), 1)

        def head_pos(i):
            head = jnp.where(i < 2 * M, jnp.where(i >= M, 1, 0), jnp.where(i >= 2 * M + T, 1, 0))
            pos = jnp.where(i < 2 * M, i - head * M, i - 2 * M - head * T + M)
            return head, pos

        rh, rp = head_pos(ri)
        ch, cp = head_pos(ci)
        vis = (rp < M) | (rp >= cp)
        fill_s[...] = jnp.where(rh == ch, jnp.where(vis, 0.0, fill_masked), -jnp.inf).astype(F32)
        ao_s[...] = jnp.zeros_like(ao_s)
        r_s[...] = jnp.full(r_s.shape, -jnp.inf, F32)

        cx.wait(); cm.wait(); cr.wait()
        wrb_s[...] = jnp.broadcast_to(wr_v[...].astype(F32).reshape(1, D), (8, D))
        lhs_s[0:M, :] = mem_v[...].astype(F32)
        lhs_s[M:L, :] = _layernorm(x_v[0:T, :].astype(F32))

        def repack(g, carry):
            for m in range(3):
                wcopy(g, m).wait()
                a = stg[3 * g + m, pl.ds(0, D // 2, stride=2), :]
                b = stg[3 * g + m, pl.ds(1, D // 2, stride=2), :]
                lo = (a & U32(0xFFFF)) | (b << 16)
                hi = (a >> 16) | (b & U32(0xFFFF0000))
                wqkv[g, :, (2 * m) * E:(2 * m + 1) * E] = pltpu.bitcast(lo, BF)
                wqkv[g, :, (2 * m + 1) * E:(2 * m + 2) * E] = pltpu.bitcast(hi, BF)
            return carry

        lax.fori_loop(0, G, repack, 0)
        for c in cwo:
            c.wait()

        def post(seg):
            r0 = pl.multiple_of(seg * T, T)
            x = x_v[pl.ds(r0, T), :].astype(F32)
            h = _rb(x + _rb(ao_s[...]))
            hn = _layernorm(h)
            h_s[pl.ds(r0, T), :] = h
            out_v[pl.ds(r0, T), :] = (h + hn).astype(BF)
            wrb = jnp.concatenate([wrb_s[...]] * (T // 8), axis=0)
            r = _rb(jnp.sum(hn * wrb, axis=-1, keepdims=True))
            lane = lax.broadcasted_iota(jnp.int32, r_s.shape, 1)
            r_s[...] = jnp.where(lane == seg, r, r_s[...])

        def order(y, m):
            a = y[:, (2 * m) * E:(2 * m + 1) * E]
            b = y[:, (2 * m + 1) * E:(2 * m + 2) * E]
            return jnp.concatenate([a[:M], b[:M], a[M:], b[M:]], axis=0)

        def step(s, carry):
            st = {}

            def qkv(g):
                y = _dot(lhs_s[...], wqkv[g])
                q = order(y, 0)
                if cfg.get('q_bf16', True):
                    q = q.astype(BF)
                st[g] = (q, order(y, 1).astype(BF), order(y, 2).astype(BF))

            def qk(g):
                q, k, v = st[g]
                sc = _dot(q, k, NT)
                fill = fill_s[...]
                sc = jnp.where(fill == 0.0, sc, fill)
                mx = jnp.max(sc, axis=-1, keepdims=True)
                p = jnp.exp2((sc - mx) * c_exp)
                l = jnp.sum(p, axis=-1, keepdims=True)
                if cfg.get('p_bf16', True):
                    p = p.astype(BF)
                st[g] = (p, l, v)

            def pv(g):
                p, l, v = st.pop(g)
                o = _dot(p, v) * pl.reciprocal(l, approx=True)
                o_s[:, (2 * g) * E:(2 * g + 1) * E] = jnp.concatenate([o[:M], o[2 * M:2 * M + T]], axis=0)
                o_s[:, (2 * g + 1) * E:(2 * g + 2) * E] = jnp.concatenate([o[M:2 * M], o[2 * M + T:]], axis=0)

            def oproj(k0, k1):
                wo = jnp.concatenate([pltpu.bitcast(wo_v[i, k0 // 2:k1 // 2, :], BF) for i in range(D // 128)], axis=1)
                return _dot(o_s[:, k0:k1], wo)

            post(jnp.maximum(s - 1, 0))
            acc = None
            for op in cfg['sched']:
                if op[0] == 'qkv':
                    qkv(op[1])
                elif op[0] == 'qk':
                    qk(op[1])
                elif op[0] == 'pv':
                    pv(op[1])
                else:
                    y = oproj(op[1] * 2 * E, op[2] * 2 * E)
                    acc = y if acc is None else acc + y
            nxt = pl.multiple_of(jnp.minimum(s + 1, NSEG - 1) * T, T)
            xn = _layernorm(x_v[pl.ds(nxt, T), :].astype(F32))
            lhs_s[M:L, :] = xn
            lhs_s[0:M, :] = acc[:M]
            ao_s[...] = acc[M:]
            return carry

        lax.fori_loop(0, NSEG, step, 0)
        post(NSEG - 1)

        r = r_s[...]
        r = jnp.where(r != r, -jnp.inf, r)
        lane = lax.broadcasted_iota(jnp.int32, r.shape, 1)
        tok = lane * T + lax.broadcasted_iota(jnp.int32, r.shape, 0)
        big = jnp.int32(1 << 30)
        ok = lane < NSEG
        m1 = jnp.max(r)
        i1 = jnp.min(jnp.where(ok & (r == m1), tok, big))
        ok2 = ok & (tok != i1)
        m2 = jnp.max(jnp.where(ok2, r, -jnp.inf))
        i2 = jnp.min(jnp.where(ok2 & (r == m2), tok, big))
        i1 = jnp.clip(i1, 0, S - 1)
        i2 = jnp.clip(i2, 0, S - 1)

        row = lax.broadcasted_iota(jnp.int32, (8, D), 0)
        hsel = jnp.where(row == 0, h_s[pl.ds(i1, 1), :], h_s[pl.ds(i2, 1), :])
        hn = _layernorm(hsel)
        rsel = jnp.where(row == 0, m1, m2)
        cg.wait(); cu.wait(); cd.wait()
        gate = _rb(_dot(hn, wg_v[...]))
        up = _rb(_dot(hn, wu_v[...]))
        act = _rb(_rb(gate * jax.nn.sigmoid(gate)) * up)
        y = _rb(_dot(act, wd_v[...]))
        y = _rb(y * _rb(jax.nn.sigmoid(rsel)))
        new = hsel + _rb(hn + y)
        for j, idx in enumerate((i1, i2)):
            b0 = pl.multiple_of((idx // 16) * 16, 16)
            rows = lax.broadcasted_iota(jnp.int32, (16, D), 0) + b0
            cur = out_v[pl.ds(b0, 16), :].astype(F32)
            out_v[pl.ds(b0, 16), :] = jnp.where(rows == idx, new[j:j + 1, :], cur).astype(BF)
        co = pltpu.make_async_copy(out_v, out_hbm, sem_m.at[11])
        co.start()
        co.wait()

    scratch = [
        pltpu.VMEM((S, D), BF),
        pltpu.VMEM((M, D), BF),
        pltpu.VMEM((D,), BF),
        pltpu.VMEM((3 * G, D, E), U32),
        pltpu.VMEM((G, D, 6 * E), BF),
        pltpu.VMEM((D // 128, H * E // 2, 128), U32),
        pltpu.VMEM((D, F), BF),
        pltpu.VMEM((D, F), BF),
        pltpu.VMEM((F, D), BF),
        pltpu.VMEM((L, D), F32),
        pltpu.VMEM((L, H * E), F32),
        pltpu.VMEM((T, D), F32),
        pltpu.VMEM((S, D), F32),
        pltpu.VMEM((S, D), BF),
        pltpu.VMEM((T, 128), F32),
        pltpu.VMEM((2 * L, 2 * L), F32),
        pltpu.VMEM((8, D), F32),
        pltpu.SemaphoreType.DMA((3 * G,)),
        pltpu.SemaphoreType.DMA((12,)),
    ]
    return kernel, scratch


def default_sched(G, d1=1, d2=2, tail=2):
    sched = []
    for t in range(G + d2):
        if t < G:
            sched.append(('qkv', t))
        else:
            k = t - G
            sched.append(('o', k * tail, (k + 1) * tail))
        if 0 <= t - d1 < G:
            sched.append(('qk', t - d1))
        if 0 <= t - d2 < G:
            sched.append(('pv', t - d2))
    sched.append(('o', d2 * tail, G))
    return sched


def build(cfg):
    @functools.partial(jax.jit, static_argnames=("A_seg_len",))
    def fn(A_x, A_mem0, A_Wq, A_Wk, A_Wv, A_Wo, A_seg_len, B_x, B_w_r, B_w_gate, B_w_up, B_w_down):
        B, S, D = A_x.shape
        _, H, E = A_Wq.shape
        M = A_mem0.shape[1]
        T = int(A_seg_len)
        F = B_w_gate.shape[1]
        c = dict(cfg)
        if 'sched' not in c:
            c['sched'] = default_sched(H // 2)
        kernel, scratch = _make_kernel(S, D, H, E, M, T, F, c)
        out = pl.pallas_call(
            kernel,
            out_shape=jax.ShapeDtypeStruct((S, D), A_x.dtype),
            in_specs=[pl.BlockSpec(memory_space=pl.ANY)] * 10,
            out_specs=pl.BlockSpec(memory_space=pl.ANY),
            scratch_shapes=scratch,
            compiler_params=pltpu.CompilerParams(vmem_limit_bytes=100 * 1024 * 1024, flags=cfg.get('flags')),
            name=cfg.get('name', 'rmt'),
        )(A_x.reshape(S, D), A_mem0.reshape(M, D), A_Wq, A_Wk, A_Wv, A_Wo.reshape(H * E, D),
          B_w_r, B_w_gate, B_w_up, B_w_down)
        return out.reshape(B, S, D)
    return fn


pallas_sequential_preLN__memory_aug_recurrent_mem_tr__moe_arch_mod__prompt_kernel = build({})
```

```python
import functools
import math

import numpy as np
import jax
import jax.numpy as jnp
from jax import lax
import jax.experimental.pallas as pl
import jax.experimental.pallas.tpu as pltpu

BF = jnp.bfloat16
F32 = jnp.float32
U32 = jnp.uint32
NN = (((1,), (0,)), ((), ()))
NT = (((1,), (1,)), ((), ()))


def _rb(v):
    return v.astype(BF).astype(F32)


def _layernorm(x):
    n = x.shape[-1]
    mean = jnp.sum(x, axis=-1, keepdims=True) * (1.0 / n)
    c = x - mean
    var = jnp.sum(c * c, axis=-1, keepdims=True) * (1.0 / n)
    eps = float(np.float32(1e-5).astype(BF))
    den = _rb(jnp.sqrt(_rb(_rb(var) + eps)))
    return _rb(x - _rb(mean)) * (1.0 / den)


def _dot(a, b, dn=NN):
    return lax.dot_general(a, b, dn, preferred_element_type=F32)


def _words(v):
    return pltpu.bitcast(v.astype(BF), U32)


def _make_kernel(S, D, H, E, M, T, F, cfg):
    G = H // 2
    L = M + T
    NSEG = S // T
    P = 8
    NPRE = cfg.get('npre', NSEG)
    N40 = NSEG - NPRE
    GROUPS = cfg.get('groups', [(1, 1), (1, 1), (2, 1), (4, 1), (4, 2)])
    U = cfg.get('unroll', 1)
    scale = float(E) ** -0.5
    fill_masked = float(np.float32(-1e9).astype(BF)) / scale
    c_exp = scale * math.log2(math.e)
    loop_only = cfg.get('loop_only', False)

    def kernel(x_hbm, mem_hbm, wq_hbm, wk_hbm, wv_hbm, wo_hbm, wr_hbm, wg_hbm, wu_hbm, wd_hbm,
               out_hbm,
               x_v, xp_v, xnp_s, mem_v, wr_v, stg, wqkv, pre, wo_v, wg_v, wu_v, wd_v,
               lhs_s, lhsb_s, o_s, ao_s, h_s, out_v, r_s, fill_s, wrb_s,
               sem_w, sem_m, sem_o):
        cxp = pltpu.make_async_copy(x_hbm.at[pl.ds(N40, NPRE), pl.ds(0, P), :], xp_v, sem_m.at[0])
        cx = pltpu.make_async_copy(x_hbm, x_v, sem_m.at[1])
        cm = pltpu.make_async_copy(mem_hbm, mem_v, sem_m.at[1])
        cr = pltpu.make_async_copy(wr_hbm, wr_v, sem_m.at[1])
        cwo = [pltpu.make_async_copy(wo_hbm.bitcast(U32).at[:, pl.ds(128 * i, 128)], wo_v.at[i], sem_m.at[1])
               for i in range(D // 128)]
        cg = pltpu.make_async_copy(wg_hbm, wg_v, sem_m.at[2])
        cu = pltpu.make_async_copy(wu_hbm, wu_v, sem_m.at[2])
        cd = pltpu.make_async_copy(wd_hbm, wd_v, sem_m.at[2])

        def wstart(i):
            g0 = sum(a * b for a, b in GROUPS[:i])
            for g in range(g0, g0 + GROUPS[i][0] * GROUPS[i][1]):
                for m, w in enumerate((wq_hbm, wk_hbm, wv_hbm)):
                    pltpu.make_async_copy(w.bitcast(U32).at[:, g, :], stg.at[3 * g + m], sem_w.at[i]).start()

        def wwait(i):
            g0 = sum(a * b for a, b in GROUPS[:i])
            blk = stg.at[pl.ds(3 * g0, 3 * GROUPS[i][0] * GROUPS[i][1])]
            pltpu.make_async_copy(blk, blk, sem_w.at[i]).wait()

        def rest_start():
            cm.start(); cr.start(); cx.start()
            for c in cwo:
                c.start()

        ahead = cfg.get('ahead', len(GROUPS) + 1)
        starts = [functools.partial(wstart, i) for i in range(len(GROUPS))] + [rest_start]
        cxp.start()
        for f in starts[:ahead]:
            f()

        ri = lax.broadcasted_iota(jnp.int32, (2 * L, 2 * L), 0)
        ci = lax.broadcasted_iota(jnp.int32, (2 * L, 2 * L), 1)

        def head_pos(i):
            n1, n2 = 2 * M, 2 * M + 2 * P
            head = jnp.where(i < n1, jnp.where(i >= M, 1, 0),
                             jnp.where(i < n2, jnp.where(i >= n1 + P, 1, 0), jnp.where(i >= n2 + T - P, 1, 0)))
            pos = jnp.where(i < n1, i - head * M,
                            jnp.where(i < n2, i - n1 - head * P + M, i - n2 - head * (T - P) + M + P))
            return head, pos

        rh, rp = head_pos(ri)
        ch, cp = head_pos(ci)
        vis = (rp < M) | (rp >= cp)
        fill_s[...] = jnp.where(rh == ch, jnp.where(vis, 0.0, fill_masked), -jnp.inf).astype(F32)
        ao_s[...] = jnp.zeros_like(ao_s)
        r_s[...] = jnp.full(r_s.shape, -jnp.inf, F32)

        cxp.wait()
        xnp_s[...] = _words(_layernorm(xp_v[...].astype(F32).reshape(NPRE * P, D)))

        def repack(i, carry, g0, n):
            for j in range(n):
                g = g0 + i * n + j
                for m in range(3):
                    a = stg[3 * g + m, pl.ds(0, D // 2, stride=2), :]
                    b = stg[3 * g + m, pl.ds(1, D // 2, stride=2), :]
                    lo = (a & U32(0xFFFF)) | (b << 16)
                    hi = (a >> 16) | (b & U32(0xFFFF0000))
                    w = jnp.concatenate([lo, hi], axis=1)
                    wqkv[3 * g + m] = w
                    y = _dot(pltpu.bitcast(xnp_s[...], BF), pltpu.bitcast(w, BF))
                    t = jnp.concatenate([y[:, :E].reshape(NPRE, P, E), y[:, E:].reshape(NPRE, P, E)], axis=1)
                    pre[3 * g + m] = _words(t.reshape(NPRE * 2 * P, E))
            return carry

        g0 = 0
        for i, (n, reps) in enumerate(GROUPS):
            wwait(i)
            if ahead + i < len(starts):
                starts[ahead + i]()
            if loop_only:
                pass
            elif reps == 1:
                repack(0, 0, g0, n)
            else:
                lax.fori_loop(0, reps, functools.partial(repack, g0=g0, n=n), 0)
            g0 += n * reps

        cg.start(); cu.start(); cd.start()
        cx.wait(); cm.wait(); cr.wait()
        for c in cwo:
            c.wait()
        wrb_s[...] = jnp.broadcast_to(wr_v[...].astype(F32).reshape(1, D), (8, D))

        def load_x(short, seg):
            if short:
                return _layernorm(x_v[seg, P:T, :].astype(F32))
            return _layernorm(x_v[seg].astype(F32))

        def load_lhs(short, mem, xn, u):
            if short:
                lhsb_s[u, 8:, :] = _words(xn[8:])
                lhsb_s[u, 0:8, :] = _words(jnp.concatenate([mem, xn[:8]], axis=0))
            else:
                lhs_s[u, M:L, :] = xn
                lhs_s[u, 0:M, :] = mem

        load_lhs(N40 == 0, mem_v[...].astype(F32), load_x(N40 == 0, 0), 0)

        def post(seg, u):
            x = x_v[seg].astype(F32)
            h = _rb(x + _rb(ao_s[u]))
            hn = _rb(_layernorm(h))
            h_s[seg] = h
            out_v[seg] = (h + hn).astype(BF)
            wrb = jnp.concatenate([wrb_s[...]] * (T // 8), axis=0)
            r = _rb(jnp.sum(hn * wrb, axis=-1, keepdims=True))
            lane = lax.broadcasted_iota(jnp.int32, r_s.shape, 1)
            r_s[...] = jnp.where(lane == seg, r, r_s[...])

        def step(s, u, short):
            st = {}

            def proj(g, m):
                lhs = pltpu.bitcast(lhsb_s[u], BF) if short else lhs_s[u]
                y = _dot(lhs, pltpu.bitcast(wqkv[3 * g + m], BF))
                a, b = y[:, :E], y[:, E:]
                if short:
                    r0 = pl.multiple_of((s - N40) * P, P)
                    t = jnp.concatenate([
                        _words(jnp.concatenate([a[:M], b[:M]], axis=0)),
                        pre[3 * g + m, pl.ds(r0, P), :],
                        _words(jnp.concatenate([a[M:], b[M:]], axis=0))], axis=0)
                    st[g, m] = pltpu.bitcast(t, BF)
                else:
                    st[g, m] = jnp.concatenate(
                        [a[:M], b[:M], a[M:M + P], b[M:M + P], a[M + P:], b[M + P:]], axis=0).astype(BF)

            def qk(g):
                sc = _dot(st.pop((g, 0)), st.pop((g, 1)), NT)
                fill = fill_s[...]
                sc = jnp.where(fill == 0.0, sc, fill)
                mx = jnp.max(sc, axis=-1, keepdims=True)
                p = jnp.exp2((sc - mx) * c_exp)
                l = jnp.sum(p, axis=-1, keepdims=True)
                if cfg.get('norm_first', False):
                    st[g] = ((p * pl.reciprocal(l, approx=True)).astype(BF), None)
                else:
                    st[g] = (p.astype(BF), l)

            def pv(g):
                p, l = st.pop(g)
                o = _dot(p, st.pop((g, 2)))
                if l is not None:
                    o = o * pl.reciprocal(l, approx=True)
                n1, n2 = 2 * M, 2 * M + 2 * P
                o_s[u, :, (2 * g) * E:(2 * g + 1) * E] = jnp.concatenate(
                    [o[:M], o[n1:n1 + P], o[n2:n2 + T - P]], axis=0)
                o_s[u, :, (2 * g + 1) * E:(2 * g + 2) * E] = jnp.concatenate(
                    [o[M:n1], o[n1 + P:n2], o[n2 + T - P:]], axis=0)

            def oproj(k0, k1):
                wo = jnp.concatenate([pltpu.bitcast(wo_v[i, k0 // 2:k1 // 2, :], BF) for i in range(D // 128)], axis=1)
                return _dot(o_s[u, :, k0:k1], wo)

            acc = None
            xn = None
            for op in cfg['sched']:
                if op[0] in 'qkv' and len(op[0]) == 1:
                    proj(op[1], 'qkv'.index(op[0]))
                elif op[0] == 'qk':
                    qk(op[1])
                elif op[0] == 'pv':
                    pv(op[1])
                elif op[0] == 'post':
                    post(jnp.maximum(s - 1, 0), u)
                elif op[0] == 'ln':
                    xn = load_x(short, jnp.minimum(s + 1, NSEG - 1))
                elif op[0] == 'o':
                    y = oproj(op[1] * 2 * E, op[2] * 2 * E)
                    acc = y if acc is None else acc + y
            load_lhs(short, acc[:M], xn, (u + 1) % U)
            ao_s[(u + 1) % U] = acc[M:]

        def steps(i, carry, short):
            for u in range(U):
                step(i * U + u, u, short)
            return carry

        if N40 > 0:
            lax.fori_loop(0, N40 // U, functools.partial(steps, short=False), 0)
            load_lhs(True, lhs_s[0, 0:M, :], load_x(True, N40), 0)
        lax.fori_loop(N40 // U, cfg.get('nsteps', NSEG) // U, functools.partial(steps, short=True), 0)
        co = pltpu.make_async_copy(out_v.at[pl.ds(0, NSEG - 1)], out_hbm.at[pl.ds(0, NSEG - 1)], sem_o.at[0])
        co.start()
        post(NSEG - 1, 0)
        cl = pltpu.make_async_copy(out_v.at[NSEG - 1], out_hbm.at[NSEG - 1], sem_o.at[1])
        cl.start()

        r = r_s[...]
        r = jnp.where(r != r, -jnp.inf, r)
        lane = lax.broadcasted_iota(jnp.int32, r.shape, 1)
        tok = lane * T + lax.broadcasted_iota(jnp.int32, r.shape, 0)
        big = jnp.int32(1 << 30)
        ok = lane < NSEG
        m1 = jnp.max(r)
        i1 = jnp.min(jnp.where(ok & (r == m1), tok, big))
        ok2 = ok & (tok != i1)
        m2 = jnp.max(jnp.where(ok2, r, -jnp.inf))
        i2 = jnp.min(jnp.where(ok2 & (r == m2), tok, big))
        i1 = jnp.clip(i1, 0, S - 1)
        i2 = jnp.clip(i2, 0, S - 1)

        row = lax.broadcasted_iota(jnp.int32, (8, D), 0)
        hsel = jnp.where(row == 0, h_s[i1 // T, pl.ds(i1 % T, 1), :], h_s[i2 // T, pl.ds(i2 % T, 1), :])
        hn = _rb(_layernorm(hsel))
        rsel = jnp.where(row == 0, m1, m2)
        cg.wait(); cu.wait(); cd.wait()
        gate = _rb(_dot(hn, wg_v[...]))
        up = _rb(_dot(hn, wu_v[...]))
        act = _rb(_rb(gate * jax.nn.sigmoid(gate)) * up)
        y = _rb(_dot(act, wd_v[...]))
        y = _rb(y * _rb(jax.nn.sigmoid(rsel)))
        new = hsel + _rb(hn + y)
        co.wait()
        cl.wait()
        for j, idx in enumerate((i1, i2)):
            rows = lax.broadcasted_iota(jnp.int32, (T, D), 0)
            cur = out_v[idx // T].astype(F32)
            out_v[idx // T] = jnp.where(rows == idx % T, new[j:j + 1, :], cur).astype(BF)
        c1 = pltpu.make_async_copy(out_v.at[i1 // T], out_hbm.at[i1 // T], sem_o.at[0])
        c2 = pltpu.make_async_copy(out_v.at[i2 // T], out_hbm.at[i2 // T], sem_o.at[1])
        c1.start()

        @pl.when(i1 // T != i2 // T)
        def _():
            c2.start()
            c2.wait()

        c1.wait()

    scratch = [
        pltpu.VMEM((NSEG, T, D), BF),
        pltpu.VMEM((NPRE, P, D), BF),
        pltpu.VMEM((NPRE * P // 2, D), U32),
        pltpu.VMEM((M, D), BF),
        pltpu.VMEM((D,), BF),
        pltpu.VMEM((3 * G, D, E), U32),
        pltpu.VMEM((3 * G, D // 2, 2 * E), U32),
        pltpu.VMEM((3 * G, NPRE * P, E), U32),
        pltpu.VMEM((D // 128, H * E // 2, 128), U32),
        pltpu.VMEM((D, F), BF),
        pltpu.VMEM((D, F), BF),
        pltpu.VMEM((F, D), BF),
        pltpu.VMEM((U, L, D), F32),
        pltpu.VMEM((U, (L - P) // 2, D), U32),
        pltpu.VMEM((U, L, H * E), F32),
        pltpu.VMEM((U, T, D), F32),
        pltpu.VMEM((NSEG, T, D), F32),
        pltpu.VMEM((NSEG, T, D), BF),
        pltpu.VMEM((T, 128), F32),
        pltpu.VMEM((2 * L, 2 * L), F32),
        pltpu.VMEM((8, D), F32),
        pltpu.SemaphoreType.DMA((len(GROUPS),)),
        pltpu.SemaphoreType.DMA((3,)),
        pltpu.SemaphoreType.DMA((2,)),
    ]
    return kernel, scratch


def default_sched(G, lv=2, dq=4, dp=5, merge_o=1, p_post=0, p_ln=52):
    main = []
    for t in range(G + lv):
        if t < G:
            main += [('k', t), ('q', t)]
        if t - lv >= 0:
            main.append(('v', t - lv))
    main += [('o', g, g + 1) for g in range(G)]
    after = {}
    for g in range(G):
        iq = main.index(('q', g)) + dq
        after.setdefault(iq, []).append(('qk', g))
        ip = max(iq + dp, main.index(('v', g)) + 3)
        after.setdefault(ip, []).append(('pv', g))
    sched = []
    for i, op in enumerate(main):
        if i == p_post:
            sched.append(('post',))
        if i == p_ln:
            sched.append(('ln',))
        if merge_o and op[0] == 'o' and sched[-1][0] == 'o':
            sched[-1] = ('o', sched[-1][1], op[2])
        else:
            sched.append(op)
        sched += after.get(i, [])
    return sched


def build(cfg):
    @functools.partial(jax.jit, static_argnames=("A_seg_len",))
    def fn(A_x, A_mem0, A_Wq, A_Wk, A_Wv, A_Wo, A_seg_len, B_x, B_w_r, B_w_gate, B_w_up, B_w_down):
        B, S, D = A_x.shape
        _, H, E = A_Wq.shape
        M = A_mem0.shape[1]
        T = int(A_seg_len)
        F = B_w_gate.shape[1]
        c = dict(cfg)
        if 'sched' not in c:
            c['sched'] = default_sched(H // 2)
        kernel, scratch = _make_kernel(S, D, H, E, M, T, F, c)
        out = pl.pallas_call(
            kernel,
            out_shape=jax.ShapeDtypeStruct((S // T, T, D), A_x.dtype),
            in_specs=[pl.BlockSpec(memory_space=pl.ANY)] * 10,
            out_specs=pl.BlockSpec(memory_space=pl.ANY),
            scratch_shapes=scratch,
            compiler_params=pltpu.CompilerParams(vmem_limit_bytes=100 * 1024 * 1024, flags=cfg.get('flags')),
            name=cfg.get('name', 'rmt'),
        )(A_x.reshape(S // T, T, D), A_mem0.reshape(M, D), A_Wq, A_Wk, A_Wv, A_Wo.reshape(H * E, D),
          B_w_r, B_w_gate, B_w_up, B_w_down)
        return out.reshape(B, S, D)
    return fn


pallas_sequential_preLN__memory_aug_recurrent_mem_tr__moe_arch_mod__prompt_kernel = build({'sched': default_sched(16, 1, 4, 5), 'ahead': 2, 'unroll': 2})
```

```python
import contextlib
import functools
import math

import numpy as np
import jax
import jax.numpy as jnp
from jax import lax
import jax.experimental.pallas as pl
import jax.experimental.pallas.tpu as pltpu

BF = jnp.bfloat16
F32 = jnp.float32
U32 = jnp.uint32
I32 = jnp.int32
NN = (((1,), (0,)), ((), ()))
NT = (((1,), (1,)), ((), ()))
INT_MIN = -(1 << 31)


def _rb(v):
    return v.astype(BF).astype(F32)


def _layernorm(x):
    n = x.shape[-1]
    mean = jnp.sum(x, axis=-1, keepdims=True) * (1.0 / n)
    c = x - mean
    var = jnp.sum(c * c, axis=-1, keepdims=True) * (1.0 / n)
    eps = float(np.float32(1e-5).astype(BF))
    den = _rb(jnp.sqrt(_rb(_rb(var) + eps)))
    return _rb(x - _rb(mean)) * (1.0 / den)


def _dot(a, b, dn=NN):
    return lax.dot_general(a, b, dn, preferred_element_type=F32)


def _words(v):
    return pltpu.bitcast(v.astype(BF), U32)


def _flip(b):
    return b ^ ((b >> 31) & 0x7FFF0000)


def _make_kernel(S, D, H, E, M, T, F, cfg):
    G = H // 2
    L = M + T
    NSEG = S // T
    KO = H * E // 2
    P = 8
    GROUPS = cfg.get('groups', (2, 3, 5, 8, 13, 17))
    XS = cfg.get('xs', 1)
    GS = cfg.get('gs', 12)
    U = cfg.get('unroll', 4)
    NIT = cfg.get('nsteps', NSEG) // U
    NF = cfg.get('nfill', 3)
    FILL = [[3 * G - 1 - (j * NF + i) for i in range(NF)] for j in range(U - 1)] + [[]]
    ROLL = sorted(w for f in FILL for w in f)
    NEARLY = (NIT - 1) * U - 1
    scale = float(E) ** -0.5
    fill_masked = float(np.float32(-1e9).astype(BF)) / scale
    c_exp = scale * math.log2(math.e)
    loop_only = cfg.get('loop_only', False)
    scope = jax.named_scope if cfg.get('prof') else (lambda n: contextlib.nullcontext())

    def kernel(x_hbm, mem_hbm, wq_hbm, wk_hbm, wv_hbm, wo_hbm, wr_hbm, wg_hbm, wu_hbm, wd_hbm,
               out_hbm,
               x_v, xp_v, xnp_s, mem_v, wr_v, stg, wqkv, pre, wo_v, wg_v, wu_v, wd_v,
               lhs_s, o_s, o2_s, ao_s, h_s, out_v, fill_s, wrb_s,
               sem_w, sem_m, sem_o):
        n = NSEG // XS
        cxp = [pltpu.make_async_copy(x_hbm.at[pl.ds(i * n, n), pl.ds(0, P), :], xp_v.at[pl.ds(i * n, n)], sem_m.at[0])
               for i in range(XS)]
        cx = [pltpu.make_async_copy(a, b, sem_m.at[1]) for a, b in ((mem_hbm, mem_v), (wr_hbm, wr_v), (x_hbm, x_v))]
        cwo = [pltpu.make_async_copy(wo_hbm.bitcast(U32).at[:, pl.ds(128 * i, 128)], wo_v.at[i], sem_m.at[2])
               for i in range(D // 128)]
        cff = [pltpu.make_async_copy(a, b, sem_m.at[0]) for a, b in ((wg_hbm, wg_v), (wu_hbm, wu_v), (wd_hbm, wd_v))]
        first = [sum(GROUPS[:i]) for i in range(len(GROUPS) + 1)]

        def wstart(i):
            for w in range(first[i], first[i + 1]):
                src = (wq_hbm, wk_hbm, wv_hbm)[w % 3]
                pltpu.make_async_copy(src.bitcast(U32).at[:, w // 3, :], stg.at[w], sem_w.at[i % 2]).start()

        def wwait(i):
            blk = stg.at[pl.ds(first[i], GROUPS[i])]
            pltpu.make_async_copy(blk, blk, sem_w.at[i % 2]).wait()

        for c in cxp:
            c.start()
        wstart(0)

        ri = lax.broadcasted_iota(I32, (2 * L, 2 * L), 0)
        ci = lax.broadcasted_iota(I32, (2 * L, 2 * L), 1)

        def head_pos(i):
            n1, n2 = 2 * M, 2 * M + 2 * P
            head = jnp.where(i < n1, jnp.where(i >= M, 1, 0),
                             jnp.where(i < n2, jnp.where(i >= n1 + P, 1, 0), jnp.where(i >= n2 + T - P, 1, 0)))
            pos = jnp.where(i < n1, i - head * M,
                            jnp.where(i < n2, i - n1 - head * P + M, i - n2 - head * (T - P) + M + P))
            return head, pos

        rh, rp = head_pos(ri)
        ch, cp = head_pos(ci)
        vis = (rp < M) | (rp >= cp)
        fill_s[...] = jnp.where(rh == ch, jnp.where(vis, 0.0, fill_masked), -jnp.inf).astype(F32)
        ao_s[0] = jnp.zeros((T, D), F32)
        o_s[U, 0:16, 0:128] = lax.bitcast_convert_type(jnp.full((16, 128), INT_MIN, I32), F32)

        with scope('w_xp'):
            pltpu.make_async_copy(xp_v, xp_v, sem_m.at[0]).wait()

        def lead(unit, w, seg0, n):
            r0 = seg0 * (P // 2)
            if not isinstance(r0, int):
                r0 = pl.multiple_of(r0, U * P // 2)
            y = _dot(pltpu.bitcast(xnp_s[pl.ds(r0, n * P // 2), :], BF), pltpu.bitcast(w, BF))
            t = jnp.concatenate([y[:, :E].reshape(n, P, E), y[:, E:].reshape(n, P, E)], axis=1)
            pre[unit, pl.ds(2 * r0, n * P), :] = _words(t.reshape(n * 2 * P, E))

        def load_x(seg):
            return _layernorm(x_v[seg, P:T, :].astype(F32))

        def store_lhs(mem, xn, u):
            lhs_s[u, 8:, :] = _words(xn[8:])
            lhs_s[u, 0:8, :] = _words(jnp.concatenate([mem, xn[:8]], axis=0))

        ng = len(GROUPS)
        for i in range(ng):
            with scope(f'w_g{i}'):
                wwait(i)
            if i + 1 < ng:
                wstart(i + 1)
            if i == ng - 2:
                for c in cx:
                    c.start()
            if i == ng - 1:
                for c in cwo:
                    c.start()
                with scope('w_x'):
                    for c in cx:
                        c.wait()
                wrb_s[...] = jnp.broadcast_to(wr_v[...].astype(F32).reshape(1, D), (8, D))
                store_lhs(mem_v[...].astype(F32), load_x(0), 0)
            for unit in range(first[i], first[i + 1]):
                if loop_only:
                    continue
                a = stg[unit, pl.ds(0, D // 2, stride=2), :]
                b = stg[unit, pl.ds(1, D // 2, stride=2), :]
                lo = (a & U32(0xFFFF)) | (b << 16)
                hi = (a >> 16) | (b & U32(0xFFFF0000))
                w = jnp.concatenate([lo, hi], axis=1)
                wqkv[unit] = w
                if i > 0:
                    lead(unit, w, 0, U if unit in ROLL else NSEG)
            if i == 0:
                s0 = 0
                for n in cfg.get('chunks', (8, 12, 16, 28)):
                    xp = xp_v[s0:s0 + n].astype(F32).reshape(n * P, D)
                    xnp_s[s0 * P // 2:(s0 + n) * P // 2, :] = _words(_layernorm(xp))
                    for unit in range(first[0], first[1]):
                        lead(unit, wqkv[unit], s0, n)
                    s0 += n

        with scope('w_wo'):
            for c in cwo:
                c.wait()

        def post(s, u, a=0, b=T):
            seg = max(s - 1, 0) if isinstance(s, int) else jnp.maximum(s - 1, 0)
            x = x_v[seg, a:b, :].astype(F32)
            h = _rb(x + _rb(ao_s[u, a:b, :]))
            hn = _rb(_layernorm(h))
            h_s[seg, a // 2:b // 2, :] = _words(h)
            out_v[seg, a:b, :] = (h + hn).astype(BF)
            wrb = jnp.concatenate([wrb_s[...]] * ((b - a) // 8), axis=0)
            r = _rb(jnp.sum(hn * wrb, axis=-1, keepdims=True))
            r = jnp.broadcast_to(r, (b - a, 128))
            key = _flip(lax.bitcast_convert_type(jnp.where(r == 0.0, 0.0, r), I32))
            key = jnp.where(r != r, INT_MIN, key)
            key = key | (S - a - seg * T - lax.broadcasted_iota(I32, (b - a, 128), 0))
            if u == 0 and not isinstance(s, int):
                key = jnp.where(s > 0, key, INT_MIN)
            slot = U + seg // 128 if cfg.get('pin', True) else U
            best = lax.bitcast_convert_type(o_s[slot, 0:16, 0:128], I32)
            b1, b2 = best[:8], best[8:]
            for j in range(0, b - a, 8):
                k = key[j:j + 8]
                b2 = jnp.maximum(b2, jnp.minimum(b1, k))
                b1 = jnp.maximum(b1, k)
            o_s[slot, 0:16, 0:128] = lax.bitcast_convert_type(jnp.concatenate([b1, b2], axis=0), F32)
            return b1, b2

        def step(s, u):
            st = {}

            def proj(g, m):
                y = _dot(pltpu.bitcast(lhs_s[u], BF), pltpu.bitcast(wqkv[3 * g + m], BF))
                a, b = y[:, :E], y[:, E:]
                t = jnp.concatenate([
                    _words(jnp.concatenate([a[:M], b[:M]], axis=0)),
                    pre[3 * g + m, pl.ds(pl.multiple_of(s * P, P), P), :],
                    _words(jnp.concatenate([a[M:], b[M:]], axis=0))], axis=0)
                st[g, m] = pltpu.bitcast(t, BF)

            def qk(g):
                sc = _dot(st.pop((g, 0)), st.pop((g, 1)), NT)
                fill = fill_s[...]
                sc = jnp.where(fill == 0.0, sc, fill)
                mx = jnp.max(sc, axis=-1, keepdims=True)
                p = jnp.exp2((sc - mx) * c_exp)
                l = jnp.sum(p, axis=-1, keepdims=True)
                st[g] = (p.astype(BF) if cfg.get('p_bf', True) else p, l)

            def pv(g):
                p, l = st.pop(g)
                o = _dot(p, st.pop((g, 2))) * pl.reciprocal(l, approx=True)
                n1, n2 = 2 * M, 2 * M + 2 * P
                dst = o_s if g < GS else o2_s
                dst[u, :, (2 * g) * E:(2 * g + 1) * E] = jnp.concatenate(
                    [o[:M], o[n1:n1 + P], o[n2:n2 + T - P]], axis=0)
                dst[u, :, (2 * g + 1) * E:(2 * g + 2) * E] = jnp.concatenate(
                    [o[M:n1], o[n1 + P:n2], o[n2 + T - P:]], axis=0)

            def oproj(k0, k1):
                wo = jnp.concatenate([pltpu.bitcast(wo_v[i, k0 // 2:k1 // 2, :], BF) for i in range(D // 128)], axis=1)
                return _dot((o_s if k0 < GS * 2 * E else o2_s)[u, :, k0:k1], wo)

            acc = None
            for op in cfg['sched']:
                if op[0] in ('q', 'k', 'v'):
                    proj(op[1], 'qkv'.index(op[0]))
                elif op[0] == 'qk':
                    qk(op[1])
                elif op[0] == 'pv':
                    pv(op[1])
                elif op[0] == 'post':
                    post(s, u, op[1], op[2])
                elif op[0] == 'o':
                    y = oproj(op[1] * 2 * E, op[2] * 2 * E)
                    acc = y if acc is None else acc + y
            store_lhs(acc[:M], load_x(jnp.minimum(s + 1, NSEG - 1)), (u + 1) % U)
            ao_s[(u + 1) % U] = acc[M:]
            for unit in FILL[u]:
                lead(unit, wqkv[unit], jnp.minimum(s - u + U, NSEG - U), U)

        co = pltpu.make_async_copy(out_v.at[pl.ds(0, NEARLY)], out_hbm.at[pl.ds(0, NEARLY)], sem_o.at[0])

        def steps(i, carry):
            @pl.when(i == NIT - 1)
            def _():
                co.start()

            @pl.when(i == 0)
            def _():
                for c in cff:
                    c.start()

            with scope('it'):
                for u in range(U):
                    step(i * U + u, u)
            return carry

        with scope('loop'):
            lax.fori_loop(0, NIT, steps, 0)
        co.wait()
        for c in cff:
            c.wait()
        b1, b2 = post(NSEG, 0)
        cl = pltpu.make_async_copy(out_v.at[pl.ds(NEARLY, NSEG - NEARLY)], out_hbm.at[pl.ds(NEARLY, NSEG - NEARLY)],
                                   sem_o.at[0])
        cl.start()

        k1 = jnp.max(b1, axis=0, keepdims=True)
        k2 = jnp.max(jnp.where(b1 == k1, b2, b1), axis=0, keepdims=True)
        i1 = jnp.clip(S - (k1[0, 0] & 0xFFFF), 0, S - 1)
        i2 = jnp.clip(S - (k2[0, 0] & 0xFFFF), 0, S - 1)
        top = lax.broadcasted_iota(I32, (8, D), 0) == 0

        def pick(i):
            w = h_s[i // T, pl.ds((i % T) // 2, 1), :]
            return lax.bitcast_convert_type(jnp.where(i % 2 == 0, w << 16, w & U32(0xFFFF0000)), F32)

        h = jnp.where(top, pick(i1), pick(i2))
        hn = _rb(_layernorm(h))
        ksel = jnp.where(top[:, :128], k1, k2) & -0x10000
        rsel = lax.bitcast_convert_type(_flip(ksel), F32)
        gate = _rb(_dot(hn, wg_v[...]))
        up = _rb(_dot(hn, wu_v[...]))
        act = _rb(gate * jax.nn.sigmoid(gate)) * up
        y = _rb(_dot(act, wd_v[...]))
        y = _rb(y * jnp.concatenate([_rb(jax.nn.sigmoid(rsel))] * (D // 128), axis=1))
        new = h + _rb(hn + y)
        with scope('w_cl'):
            cl.wait()
        for j, idx in enumerate((i1, i2)):
            rows = lax.broadcasted_iota(I32, (T, D), 0)
            cur = out_v[idx // T].astype(F32)
            out_v[idx // T] = jnp.where(rows == idx % T, new[j:j + 1, :], cur).astype(BF)
        c1 = pltpu.make_async_copy(out_v.at[i1 // T], out_hbm.at[i1 // T], sem_o.at[0])
        c2 = pltpu.make_async_copy(out_v.at[i2 // T], out_hbm.at[i2 // T], sem_o.at[1])
        c1.start()

        @pl.when(i1 // T != i2 // T)
        def _():
            c2.start()
            c2.wait()

        with scope('w_c1'):
            c1.wait()

    scratch = [
        pltpu.VMEM((NSEG, T, D), BF),
        pltpu.VMEM((NSEG, P, D), BF),
        pltpu.VMEM((NSEG * P // 2, D), U32),
        pltpu.VMEM((M, D), BF),
        pltpu.VMEM((D,), BF),
        pltpu.VMEM((3 * G, D, E), U32),
        pltpu.VMEM((3 * G, D // 2, 2 * E), U32),
        pltpu.VMEM((3 * G, NSEG * P, E), U32),
        pltpu.VMEM((D // 128, KO, 128), U32),
        pltpu.VMEM((D, F), BF),
        pltpu.VMEM((D, F), BF),
        pltpu.VMEM((F, D), BF),
        pltpu.VMEM((U, (L - P) // 2, D), U32),
        pltpu.VMEM((U + 1, L, H * E), F32),
        pltpu.VMEM((U, L, H * E), F32),
        pltpu.VMEM((U, T, D), F32),
        pltpu.VMEM((NSEG, T // 2, D), U32),
        pltpu.VMEM((NSEG, T, D), BF),
        pltpu.VMEM((2 * L, 2 * L), F32),
        pltpu.VMEM((8, D), F32),
        pltpu.SemaphoreType.DMA((2,)),
        pltpu.SemaphoreType.DMA((3,)),
        pltpu.SemaphoreType.DMA((2,)),
    ]
    return kernel, scratch


def default_sched(G, lv=1, dq=4, dp=5, p_post=(54, 59), order='kqv', seed=0, jit=0):
    rng = np.random.RandomState(seed)
    main = []
    for t in range(G + lv):
        for c in order:
            g = t - lv if c == 'v' else t
            if 0 <= g < G:
                main.append((c, g))
    main += [('o', g, g + 1) for g in range(G)]
    after = {}
    for g in range(G):
        iq = max(main.index(('q', g)), main.index(('k', g))) + dq + rng.randint(0, jit + 1)
        after.setdefault(iq, []).append(('qk', g))
        ip = max(iq + dp + rng.randint(0, jit + 1), main.index(('v', g)) + 3)
        after.setdefault(ip, []).append(('pv', g))
    sched = []
    for i, op in enumerate(main):
        for j, pp in enumerate(p_post):
            if i == pp:
                sched.append(('post', j * 32 // len(p_post), (j + 1) * 32 // len(p_post)))
        sched.append(op)
        sched += after.get(i, [])
    return sched


def build(cfg):
    @functools.partial(jax.jit, static_argnames=("A_seg_len",))
    def fn(A_x, A_mem0, A_Wq, A_Wk, A_Wv, A_Wo, A_seg_len, B_x, B_w_r, B_w_gate, B_w_up, B_w_down):
        B, S, D = A_x.shape
        _, H, E = A_Wq.shape
        M = A_mem0.shape[1]
        T = int(A_seg_len)
        F = B_w_gate.shape[1]
        c = dict(cfg)
        if 'sched' not in c:
            c['sched'] = default_sched(H // 2)
        kernel, scratch = _make_kernel(S, D, H, E, M, T, F, c)
        out = pl.pallas_call(
            kernel,
            out_shape=jax.ShapeDtypeStruct((S // T, T, D), A_x.dtype),
            in_specs=[pl.BlockSpec(memory_space=pl.ANY)] * 10,
            out_specs=pl.BlockSpec(memory_space=pl.ANY),
            scratch_shapes=scratch,
            compiler_params=pltpu.CompilerParams(vmem_limit_bytes=100 * 1024 * 1024, flags=cfg.get('flags')),
            name=cfg.get('name', 'rmt'),
        )(A_x.reshape(S // T, T, D), A_mem0.reshape(M, D), A_Wq, A_Wk, A_Wv, A_Wo.reshape(H * E, D),
          B_w_r, B_w_gate, B_w_up, B_w_down)
        return out.reshape(B, S, D)
    return fn


pallas_sequential_preLN__memory_aug_recurrent_mem_tr__moe_arch_mod__prompt_kernel = build({'sched': default_sched(16, 0, 2, 5, (56, 59), 'vkq')})
```

```python
import functools
import math

import numpy as np
import jax
import jax.numpy as jnp
from jax import lax
import jax.experimental.pallas as pl
import jax.experimental.pallas.tpu as pltpu

BF = jnp.bfloat16
F32 = jnp.float32
U32 = jnp.uint32
I32 = jnp.int32
INT_MIN = -(1 << 31)
_NN = (((1,), (0,)), ((), ()))
_NT = (((1,), (1,)), ((), ()))


def _rb(v):
    return v.astype(BF).astype(F32)


def _layernorm(x):
    n = x.shape[-1]
    mean = jnp.sum(x, axis=-1, keepdims=True) * (1.0 / n)
    c = x - mean
    var = jnp.sum(c * c, axis=-1, keepdims=True) * (1.0 / n)
    eps = float(np.float32(1e-5).astype(BF))
    den = _rb(jnp.sqrt(_rb(_rb(var) + eps)))
    return _rb(x - _rb(mean)) * (1.0 / den)


def _dot(a, b, dn=_NN):
    return lax.dot_general(a, b, dn, preferred_element_type=F32)


def _words(v):
    return pltpu.bitcast(v.astype(BF), U32)


def _rows(w):
    return pltpu.bitcast(w, BF)


def _flip(b):
    return b ^ ((b >> 31) & 0x7FFF0000)


def _step_order(G):
    main = []
    for g in range(G + 1):
        if g < G:
            main += [('k', g), ('q', g)]
        if g > 0:
            main.append(('v', g - 1))
    main += [('o', g) for g in range(G)]
    after = {}
    for g in range(G):
        i = main.index(('q', g)) + 3
        after.setdefault(i, []).append(('qk', g))
        after.setdefault(max(i + 4, main.index(('v', g)) + 3), []).append(('pv', g))
    before = {('o', G // 2): [('post', 0)], ('o', G // 2 + 3): [('post', 1)]}
    order = []
    for i, op in enumerate(main):
        order += before.get(op, []) + [op] + after.get(i, [])
    return order


def _make_kernel(S, D, H, E, M, T, F):
    G = H // 2
    NW = 3 * G
    GA = 3 * G // 4
    L = M + T
    P = 8
    U = 4
    NSEG = S // T
    NIT = NSEG // U
    NF = 2
    FILL = [[NW - 1 - (j * NF + i) for i in range(NF)] for j in range(U - 1)] + [[]]
    NROLL = NF * (U - 1)
    GROUPS = (2, 3, 5, 8, 14, 16)
    CHUNKS = (2, 3, 4, 7)
    NEARLY = (NIT - 1) * U - 1
    assert (M, T, E) == (8, 32, 128) and D % 128 == 0 and S < (1 << 16)
    assert sum(GROUPS) == NW and sum(CHUNKS) == NIT and NIT * U * T == S
    first = [sum(GROUPS[:i]) for i in range(len(GROUPS) + 1)]
    scale = float(E) ** -0.5
    masked = float(np.float32(-1e9).astype(BF)) / scale
    c_exp = scale * math.log2(math.e)
    n1, n2 = 2 * M, 2 * M + 2 * P

    def kernel(x_hbm, mem_hbm, wq_hbm, wk_hbm, wv_hbm, wo_hbm, wr_hbm, wg_hbm, wu_hbm, wd_hbm, out_hbm,
               wqkv, pre, stg, wg_v, wu_v, wd_v, x_v, xp_v, xnp_s, h_s, out_v, oa_s, ob_s, wo_v,
               lhs_s, ao_s, wrb_s, fill_s, mem_v, wr_v, sems):
        copy = pltpu.make_async_copy
        c_lead = copy(x_hbm.at[:, pl.ds(0, P), :], xp_v, sems.at[1])
        c_x = [copy(a, b, sems.at[1]) for a, b in ((mem_hbm, mem_v), (wr_hbm, wr_v), (x_hbm, x_v))]
        c_wo = [copy(wo_hbm.bitcast(U32).at[:, pl.ds(128 * i, 128)], wo_v.at[i], sems.at[0])
                for i in range(D // 128)]
        c_ffn = [copy(a, b, sems.at[1]) for a, b in ((wg_hbm, wg_v), (wu_hbm, wu_v), (wd_hbm, wd_v))]

        def start_weights(i):
            for w in range(first[i], first[i + 1]):
                src = (wq_hbm, wk_hbm, wv_hbm)[w % 3]
                copy(src.bitcast(U32).at[:, w // 3, :], stg.at[w], sems.at[0]).start()

        def wait_weights(i):
            blk = stg.at[pl.ds(first[i], GROUPS[i])]
            copy(blk, blk, sems.at[0]).wait()

        c_lead.start()
        start_weights(0)

        def head_pos(i):
            head = jnp.where(i < n1, jnp.where(i >= M, 1, 0),
                             jnp.where(i < n2, jnp.where(i >= n1 + P, 1, 0), jnp.where(i >= n2 + T - P, 1, 0)))
            pos = jnp.where(i < n1, i - head * M,
                            jnp.where(i < n2, i - n1 - head * P + M, i - n2 - head * (T - P) + M + P))
            return head, pos

        rh, rp = head_pos(lax.broadcasted_iota(I32, (2 * L, 2 * L), 0))
        ch, cp = head_pos(lax.broadcasted_iota(I32, (2 * L, 2 * L), 1))
        visible = (rp < M) | (rp >= cp)
        fill_s[...] = jnp.where(rh == ch, jnp.where(visible, 0.0, masked), -jnp.inf).astype(F32)
        ao_s[0] = jnp.zeros((T, D), F32)
        oa_s[U, 0:16, 0:128] = lax.bitcast_convert_type(jnp.full((16, 128), INT_MIN, I32), F32)
        c_lead.wait()

        def lead(unit, w, it0, n):
            y = _dot(_rows(xnp_s[pl.ds(it0, n)].reshape(n * U * P // 2, D)), _rows(w))
            t = jnp.concatenate([y[:, :E].reshape(n * U, P, E), y[:, E:].reshape(n * U, P, E)], axis=1)
            pre[unit, pl.ds(it0, n)] = _words(t.reshape(n * U * 2 * P, E)).reshape(n, U * P, E)

        def store_lhs(mem, seg, u):
            xn = _layernorm(x_v[seg, P:T, :].astype(F32))
            lhs_s[u, 8:, :] = _words(xn[8:])
            lhs_s[u, :8, :] = _words(jnp.concatenate([mem, xn[:8]], axis=0))

        last = len(GROUPS) - 1
        for i in range(last + 1):
            wait_weights(i)
            if i < last:
                start_weights(i + 1)
            if i == last - 1:
                for c in c_x:
                    c.start()
            if i == last:
                for c in c_wo:
                    c.start()
                for c in c_x:
                    c.wait()
                wrb_s[...] = jnp.broadcast_to(wr_v[...].astype(F32).reshape(1, D), (8, D))
                store_lhs(mem_v[...].astype(F32), 0, 0)
            for unit in range(first[i], first[i + 1]):
                a = stg[unit, pl.ds(0, D // 2, stride=2), :]
                b = stg[unit, pl.ds(1, D // 2, stride=2), :]
                w = jnp.concatenate([(a & U32(0xFFFF)) | (b << 16), (a >> 16) | (b & U32(0xFFFF0000))], axis=1)
                wqkv[unit] = w
                if i > 0:
                    lead(unit, w, 0, NIT if unit < NW - NROLL else 1)
            if i == 0:
                it0 = 0
                for n in CHUNKS:
                    xp = xp_v[it0 * U:(it0 + n) * U].astype(F32).reshape(n * U * P, D)
                    xnp_s[it0:it0 + n] = _words(_layernorm(xp)).reshape(n, U * P // 2, D)
                    for unit in range(first[1]):
                        lead(unit, wqkv[unit], it0, n)
                    it0 += n
        for c in c_wo:
            c.wait()

        def post(seg, u, a, b, live=None):
            h = _rb(x_v[seg, a:b, :].astype(F32) + _rb(ao_s[u, a:b, :]))
            hn = _rb(_layernorm(h))
            h_s[seg, a // 2:b // 2, :] = _words(h)
            out_v[seg, a:b, :] = (h + hn).astype(BF)
            wr = jnp.concatenate([wrb_s[...]] * ((b - a) // 8), axis=0)
            r = jnp.broadcast_to(_rb(jnp.sum(hn * wr, axis=-1, keepdims=True)), (b - a, 128))
            key = _flip(lax.bitcast_convert_type(jnp.where(r == 0.0, 0.0, r), I32))
            key = jnp.where(r != r, INT_MIN, key)
            key = key | (S - a - seg * T - lax.broadcasted_iota(I32, (b - a, 128), 0))
            if live is not None:
                key = jnp.where(live, key, INT_MIN)
            slot = U + seg // (2 * NSEG)
            best = lax.bitcast_convert_type(oa_s[slot, 0:16, 0:128], I32)
            b1, b2 = best[:8], best[8:]
            for j in range(0, b - a, 8):
                b2 = jnp.maximum(b2, jnp.minimum(b1, key[j:j + 8]))
                b1 = jnp.maximum(b1, key[j:j + 8])
            oa_s[slot, 0:16, 0:128] = lax.bitcast_convert_type(jnp.concatenate([b1, b2], axis=0), F32)
            return b1, b2

        def step(i, u):
            s = i * U + u
            st = {}
            acc = None
            for op, g in _step_order(G):
                o_ref, c0 = (oa_s, g * 2 * E) if g < GA else (ob_s, (g - GA) * 2 * E)
                if op in ('q', 'k', 'v'):
                    unit = 3 * g + 'qkv'.index(op)
                    y = _dot(_rows(lhs_s[u]), _rows(wqkv[unit]))
                    a, b = y[:, :E], y[:, E:]
                    st[op, g] = _rows(jnp.concatenate([
                        _words(jnp.concatenate([a[:M], b[:M]], axis=0)),
                        pre[unit, i, u * P:(u + 1) * P, :],
                        _words(jnp.concatenate([a[M:], b[M:]], axis=0))], axis=0))
                elif op == 'qk':
                    fill = fill_s[...]
                    sc = jnp.where(fill == 0.0, _dot(st.pop(('q', g)), st.pop(('k', g)), _NT), fill)
                    p = jnp.exp2((sc - jnp.max(sc, axis=-1, keepdims=True)) * c_exp)
                    st['p', g] = (p.astype(BF), jnp.sum(p, axis=-1, keepdims=True))
                elif op == 'pv':
                    p, den = st.pop(('p', g))
                    inv = pltpu.reciprocal(den, approx=True)
                    inv = inv * (2.0 - den * inv)
                    o = _dot(p, st.pop(('v', g))) * inv
                    o_ref[u, :, c0:c0 + E] = jnp.concatenate([o[:M], o[n1:n1 + P], o[n2:n2 + T - P]], axis=0)
                    o_ref[u, :, c0 + E:c0 + 2 * E] = jnp.concatenate([o[M:n1], o[n1 + P:n2], o[n2 + T - P:]], axis=0)
                elif op == 'o':
                    wo = jnp.concatenate([_rows(wo_v[c, g * E:(g + 1) * E, :]) for c in range(D // 128)], axis=1)
                    y = _dot(o_ref[u, :, c0:c0 + 2 * E], wo)
                    acc = y if acc is None else acc + y
                else:
                    post(jnp.maximum(s - 1, 0), u, g * T // 2, (g + 1) * T // 2, s > 0 if u == 0 else None)
            store_lhs(acc[:M], jnp.minimum(s + 1, NSEG - 1), (u + 1) % U)
            ao_s[(u + 1) % U] = acc[M:]
            for unit in FILL[u]:
                lead(unit, wqkv[unit], jnp.minimum(i + 1, NIT - 1), 1)

        c_early = copy(out_v.at[pl.ds(0, NEARLY)], out_hbm.at[pl.ds(0, NEARLY)], sems.at[0])
        c_late = copy(out_v.at[pl.ds(NEARLY, NSEG - NEARLY)], out_hbm.at[pl.ds(NEARLY, NSEG - NEARLY)], sems.at[0])

        def iteration(i, carry):
            @pl.when(i == NIT - 1)
            def _():
                c_early.start()

            @pl.when(i == 0)
            def _():
                for c in c_ffn:
                    c.start()

            for u in range(U):
                step(i, u)
            return carry

        lax.fori_loop(0, NIT, iteration, 0)
        c_early.wait()
        for c in c_ffn:
            c.wait()
        b1, b2 = post(NSEG - 1, 0, 0, T)
        c_late.start()

        k1 = jnp.max(b1, axis=0, keepdims=True)
        k2 = jnp.max(jnp.where(b1 == k1, b2, b1), axis=0, keepdims=True)
        i1 = jnp.clip(S - (k1[0, 0] & 0xFFFF), 0, S - 1)
        i2 = jnp.clip(S - (k2[0, 0] & 0xFFFF), 0, S - 1)
        top = lax.broadcasted_iota(I32, (8, D), 0) == 0

        def h_row(i):
            w = h_s[i // T, pl.ds((i % T) // 2, 1), :]
            return lax.bitcast_convert_type(jnp.where(i % 2 == 0, w << 16, w & U32(0xFFFF0000)), F32)

        h = jnp.where(top, h_row(i1), h_row(i2))
        hn = _rb(_layernorm(h))
        r = lax.bitcast_convert_type(_flip(jnp.where(top[:, :128], k1, k2) & -0x10000), F32)
        gate = _rb(_dot(hn, wg_v[...]))
        up = _rb(_dot(hn, wu_v[...]))
        y = _rb(_dot(_rb(gate * jax.nn.sigmoid(gate)) * up, wd_v[...]))
        y = _rb(y * jnp.concatenate([_rb(jax.nn.sigmoid(r))] * (D // 128), axis=1))
        routed = h + _rb(hn + y)
        c_late.wait()
        for j, idx in enumerate((i1, i2)):
            row = lax.broadcasted_iota(I32, (T, D), 0)
            cur = out_v[idx // T].astype(F32)
            out_v[idx // T] = jnp.where(row == idx % T, routed[j:j + 1, :], cur).astype(BF)
        c1 = copy(out_v.at[i1 // T], out_hbm.at[i1 // T], sems.at[0])
        c2 = copy(out_v.at[i2 // T], out_hbm.at[i2 // T], sems.at[1])
        c1.start()

        @pl.when(i1 // T != i2 // T)
        def _():
            c2.start()
            c2.wait()

        c1.wait()

    scratch = [
        pltpu.VMEM((NW, D // 2, 2 * E), U32),
        pltpu.VMEM((NW, NIT, U * P, E), U32),
        pltpu.VMEM((NW, D, E), U32),
        pltpu.VMEM((D, F), BF),
        pltpu.VMEM((D, F), BF),
        pltpu.VMEM((F, D), BF),
        pltpu.VMEM((NSEG, T, D), BF),
        pltpu.VMEM((NSEG, P, D), BF),
        pltpu.VMEM((NIT, U * P // 2, D), U32),
        pltpu.VMEM((NSEG, T // 2, D), U32),
        pltpu.VMEM((NSEG, T, D), BF),
        pltpu.VMEM((U + 1, L, GA * 2 * E), F32),
        pltpu.VMEM((U, L, (G - GA) * 2 * E), F32),
        pltpu.VMEM((D // 128, H * E // 2, 128), U32),
        pltpu.VMEM((U, (L - P) // 2, D), U32),
        pltpu.VMEM((U, T, D), F32),
        pltpu.VMEM((8, D), F32),
        pltpu.VMEM((2 * L, 2 * L), F32),
        pltpu.VMEM((M, D), BF),
        pltpu.VMEM((D,), BF),
        pltpu.SemaphoreType.DMA((2,)),
    ]
    return kernel, scratch


@functools.partial(jax.jit, static_argnames=("A_seg_len",))
def pallas_sequential_preLN__memory_aug_recurrent_mem_tr__moe_arch_mod__prompt_kernel(
    A_x, A_mem0, A_Wq, A_Wk, A_Wv, A_Wo, A_seg_len, B_x, B_w_r, B_w_gate, B_w_up, B_w_down,
):
    del B_x
    B, S, D = A_x.shape
    _, H, E = A_Wq.shape
    M = A_mem0.shape[1]
    T = int(A_seg_len)
    F = B_w_gate.shape[1]
    assert B == 1
    kernel, scratch = _make_kernel(S, D, H, E, M, T, F)
    out = pl.pallas_call(
        kernel,
        out_shape=jax.ShapeDtypeStruct((S // T, T, D), A_x.dtype),
        in_specs=[pl.BlockSpec(memory_space=pl.ANY)] * 10,
        out_specs=pl.BlockSpec(memory_space=pl.ANY),
        scratch_shapes=scratch,
        compiler_params=pltpu.CompilerParams(
            vmem_limit_bytes=100 * 1024 * 1024,
            flags={"XLA_TPU_EVENLY_DISTRIBUTE_CRITICAL_NODES": True}),
        name="rmt_mod",
    )(A_x.reshape(S // T, T, D), A_mem0.reshape(M, D), A_Wq, A_Wk, A_Wv, A_Wo.reshape(H * E, D),
      B_w_r, B_w_gate, B_w_up, B_w_down)
    return out.reshape(B, S, D)
```
